```python
import os as _os
_os.environ.setdefault("JAX_PLATFORMS", "cpu")
import jax
import jax.numpy as jnp

def _softmax(x, axis=-1):
    return jax.nn.softmax(x, axis=axis)
def _gelu(x):
    return jax.nn.gelu(x, approximate=True)
def _silu(x):
    return jax.nn.silu(x)
def _sigmoid(x):
    return jax.nn.sigmoid(x)
def _layernorm(x, axis=-1, eps=1e-5):
    m = jnp.mean(x, axis=axis, keepdims=True)
    v = jnp.var(x, axis=axis, keepdims=True)
    return (x - m) / jnp.sqrt(v + eps)
def _scatter_add(tgt, idx, src, axis=0):
    return tgt.at[idx].add(src)
def _segment_sum(src, seg, n):
    return jax.ops.segment_sum(src, seg, n)
class _Rng:
    def __init__(self, key):
        self._k = key
    def _next(self):
        self._k, sub = jax.random.split(self._k)
        return sub
    def normal(self, shape):
        return jax.random.normal(self._next(), shape, dtype=jnp.bfloat16)
    def randint(self, lo, hi, shape):
        return jax.random.randint(self._next(), shape, lo, hi, dtype=jnp.int32)
    def uniform(self, shape, lo=0.0, hi=1.0):
        return jax.random.uniform(self._next(), shape, jnp.bfloat16, lo, hi)
    def permutation(self, n):
        return jax.random.permutation(self._next(), n)


kernel_name = 'sequential_preLN__ssm_conv_h3__mixer_channel_mlp__prompt'

def setup_inputs():
    _rng = _Rng(jax.random.key(int.from_bytes(__import__("os").urandom(4), "little")))
    _w = (lambda a: (lambda t: t.astype(jnp.bfloat16) if jnp.issubdtype(t.dtype, jnp.floating) else t)(jnp.asarray(a)))
    def _A_setup():
        B, S, D = 1, 2048, 448
        ks = 4
        return {
            "q": _w((lambda *s: _rng.normal(s) * 0.05)(B, S, D)),
            "k": _w((lambda *s: _rng.normal(s) * 0.05)(B, S, D)),
            "v": _w((lambda *s: _rng.normal(s) * 0.05)(B, S, D)),
            "shift_k": _w((lambda *s: _rng.normal(s) * 0.05)(D, ks) * 0.5),
            "ssm_k": _w((lambda *s: _rng.normal(s) * 0.05)(D, S) * (1.0 / S ** 0.5)),
            "ssm_D": _w((lambda *s: _rng.normal(s) * 0.05)(D)),
        }
    _A_in = _A_setup()

    def _B_setup():
        B, S, D, F = 1, 2048, 448, 1792
        return {
            "x": _w((lambda *s: _rng.normal(s) * 0.05)(B, S, D)),
            "w1": _w((lambda *s: _rng.normal(s) * 0.2)(D, F) * (D ** -0.5)),
            "b1": _w((lambda *s: _rng.normal(s) * 0.2)(F)),
            "w2": _w((lambda *s: _rng.normal(s) * 0.2)(F, D) * (F ** -0.5)),
            "b2": _w((lambda *s: _rng.normal(s) * 0.05)(D)),
        }
    _B_in = _B_setup()

    return {
        "A_q": _A_in["q"],
        "A_k": _A_in["k"],
        "A_v": _A_in["v"],
        "A_shift_k": _A_in["shift_k"],
        "A_ssm_k": _A_in["ssm_k"],
        "A_ssm_D": _A_in["ssm_D"],
        "B_x": _B_in["x"],
        "B_w1": _B_in["w1"],
        "B_b1": _B_in["b1"],
        "B_w2": _B_in["w2"],
        "B_b2": _B_in["b2"],
    }

def reference(A_q, A_k, A_v, A_shift_k, A_ssm_k, A_ssm_D, B_x, B_w1, B_b1, B_w2, B_b2):
    def _A_ref(q, k, v, shift_k, ssm_k, ssm_D):
        B, S, D = q.shape
        ks = shift_k.shape[-1]
        k_pad = jnp.pad(k, ((0, 0), (ks - 1, 0), (0, 0)))
        k_shift = jnp.zeros_like(k)
        for t in range(ks):
            k_shift = k_shift + k_pad[:, t:t + S, :] * shift_k[:, ks - 1 - t][None, None, :]
        kv = k_shift * v
        L = 2 * S
        kv_pad = jnp.pad(kv, ((0, 0), (0, S), (0, 0)))
        kf_pad = jnp.pad(ssm_k, ((0, 0), (0, S)))
        kv_f = (lambda x, axes=(-2,-1): jnp.fft.rfft2(x.astype(jnp.float32), axes=axes))(kv_pad[:, None, :, :], axes=(1, 2))
        kf_f = (lambda x, axes=(-2,-1): jnp.fft.rfft2(x.astype(jnp.float32), axes=axes))(kf_pad[:, None, :], axes=(1, 2))
        kf_f = (lambda x, *d: x.transpose(*d))(kf_f, 1, 2, 0)
        y_f = kv_f * kf_f[None, :, :, :]
        y = (lambda x, s, axes=(-2,-1): jnp.fft.irfft2(x, s=s, axes=axes).astype(jnp.bfloat16))(y_f, (1, L), axes=(1, 2))[:, 0, :S, :]
        y = y + kv * ssm_D[None, None, :]
        return q * y

    def _B_ref(x, w1, b1, w2, b2):
        y = _layernorm(x, axis=-1)
        h = _gelu(jnp.einsum("bsd,df->bsf", y, w1) + b1)
        return jnp.einsum("bsf,fd->bsd", h, w2) + b2

    x = A_q
    h = x + _A_ref(_layernorm(x, axis=-1), A_k, A_v, A_shift_k, A_ssm_k, A_ssm_D)
    h2 = h + _B_ref(_layernorm(h, axis=-1), B_w1, B_b1, B_w2, B_b2)
    return h2
```

```python
import functools
import math

import jax
import jax.numpy as jnp
import numpy as np
import jax.experimental.pallas as pl
import jax.experimental.pallas.tpu as pltpu

_B = 128
_EPS = 1e-5


def _dft_mats():
    j = np.arange(_B, dtype=np.float64)
    th = 2.0 * np.pi * (j[:, None] + 0.25) * j[None, :] / _B
    fwd = np.concatenate([np.cos(th).T, -np.sin(th).T], axis=1)
    inv = np.concatenate([np.cos(th), -np.sin(th)], axis=0) / _B
    return fwd.astype(np.float32), inv.astype(np.float32)


def _ln(x):
    m = jnp.mean(x, axis=0, keepdims=True)
    xc = x - m
    v = jnp.mean(xc * xc, axis=0, keepdims=True)
    return xc * jax.lax.rsqrt(v + _EPS)


def _gelu(x):
    c0 = math.sqrt(2.0 / math.pi)
    u = x * (c0 + (c0 * 0.044715) * (x * x))
    hx = 0.5 * x
    return hx * jnp.tanh(u) + hx


def _kernel(q_hbm, k_hbm, v_hbm, shift_ref, sk_hbm, ssmd_ref, w1_hbm, b1_ref, w2_hbm, b2_ref,
            fwd_ref, inv_ref, out_hbm,
            qv, kb, vb, skb, w1v, w1t, w2v, w2t, gb, rows, cols, xh, kh, qs, hbuf, ybuf, ob, isem, osem,
            *, S, D, DP, F, KS, CH):
    NB = S // _B
    NS = NB // 2
    NC = S // CH
    bf, f32 = jnp.bfloat16, jnp.float32

    def in_copies(i):
        r = pl.ds(i * CH, CH)
        return (
            pltpu.make_async_copy(k_hbm.at[:, r], kb.at[:, pl.ds(_B + i * CH, CH)], isem.at[3 * i]),
            pltpu.make_async_copy(v_hbm.at[:, r], vb.at[:, r], isem.at[3 * i + 1]),
            pltpu.make_async_copy(sk_hbm.at[:, r], skb.at[:, r], isem.at[3 * i + 2]),
        )

    w1_cp = pltpu.make_async_copy(w1_hbm, w1v.at[0:D], isem.at[3 * NC])
    w2_cp = pltpu.make_async_copy(w2_hbm, w2v, isem.at[3 * NC + 1])
    q_cp = pltpu.make_async_copy(q_hbm, qv, isem.at[3 * NC + 2])

    for i in range(NC):
        for cp in in_copies(i):
            cp.start()
    w1_cp.start()
    q_cp.start()
    w2_cp.start()

    rows[...] = jnp.zeros(rows.shape, f32)
    rows[0:KS, 0:D] = shift_ref[...].astype(f32)
    rows[KS:KS + 1, 0:D] = ssmd_ref[...].astype(f32).reshape(1, D)
    rows[KS + 1:KS + 2, 0:D] = b2_ref[...].astype(f32).reshape(1, D)
    rt = rows[...].T
    for j in range(KS + 2):
        cols[j] = jnp.broadcast_to(rt[0:D, j:j + 1], (D, _B))
    kb[:, 0:_B] = jnp.zeros((D, _B), bf)
    pad_rows = jax.lax.broadcasted_iota(jnp.int32, (DP - D, 2 * _B), 0)
    for sl in range(2):
        ybuf[sl, D:DP, :] = (pad_rows == 0).astype(bf)
    w1v[D:DP, :] = jnp.zeros((DP - D, F), bf)
    w1v[D:D + 16, :] = jnp.where(
        jax.lax.broadcasted_iota(jnp.int32, (16, F), 0) == 0,
        b1_ref[...].astype(f32).reshape(1, F), 0.0).astype(bf)

    def p1(i, _):
        for cp in in_copies(i):
            cp.wait()
        fwd = fwd_ref[...]
        prev = qs[0]
        r0 = pl.multiple_of(i * CH, CH)
        kk = kb[:, pl.ds(r0, _B + CH)].astype(f32)
        rolled = [kk] + [pltpu.roll(kk, j, 1) for j in range(1, KS)]
        for jb in range(CH // _B):
            c = i * (CH // _B) + jb
            r = pl.ds(pl.multiple_of(c * _B, _B), _B)
            ksft = None
            for j in range(KS):
                t = rolled[j][:, _B * (jb + 1):_B * (jb + 2)].astype(f32) * cols[j]
                ksft = t if ksft is None else ksft + t
            kv = (ksft * vb[:, r].astype(f32)).astype(bf)
            vb[:, r] = kv
            xh[c] = jnp.dot(kv, fwd, preferred_element_type=f32)
            ks = jnp.dot(skb[:, r], fwd, preferred_element_type=f32)
            kh[c, :, 0:_B] = ks[:, 0:_B] - prev[:, _B:]
            kh[c, :, _B:] = ks[:, _B:] + prev[:, 0:_B]
            prev = ks
        qs[0] = prev
        return 0

    qs[0] = jnp.zeros((D, 2 * _B), f32)
    jax.lax.fori_loop(0, NC, p1, 0)

    w1_cp.wait()
    w1t[...] = w1v[...].T
    FR, CC, FC, OC = 16, 64, 256, 448

    def conv_parts(s, slot):
        idx = []
        for p in range(NB + 1):
            first = p <= s
            m = jnp.where(first, p, p - s - 1)
            c = jnp.where(first, s, NB - 1 - s)
            idx.append((m, c - m, jnp.where(first, 0, 1)))
        re, im = slice(0, _B), slice(_B, 2 * _B)
        ra = pl.ds(pl.multiple_of(s * _B, _B), _B)
        rb = pl.ds(pl.multiple_of((NB - 1 - s) * _B, _B), _B)
        st = {}

        def two(ref, ch):
            return jnp.concatenate([ref[ch, ra], ref[ch, rb]], axis=1).astype(f32)

        def stats():
            x = two(qv, slice(None))
            m = jnp.mean(x, axis=0, keepdims=True)
            xc = x - m
            st["m"] = m
            st["r"] = jax.lax.rsqrt(jnp.mean(xc * xc, axis=0, keepdims=True) + _EPS)

        def mac(d0):
            ch = slice(d0, d0 + FR)
            are = aim = None
            for p, (m, n, sl) in enumerate(idx):
                kr, ki = kh[m, ch, re], kh[m, ch, im]
                xr, xi = xh[n, ch, re], xh[n, ch, im]
                tr = kr * xr - ki * xi
                ti = kr * xi + ki * xr
                are = tr if are is None else are + tr
                aim = ti if aim is None else aim + ti
                if p < NS or p == NB:
                    qs[sl, ch, re] = are
                    qs[sl, ch, im] = aim

        def back(d0):
            ch = slice(d0, d0 + CC)
            qa = qs[0, ch, :]
            qb = qs[1, ch, :] - qa
            y = jnp.dot(jnp.concatenate([qa, qb], axis=0).astype(bf), inv_ref[...],
                        preferred_element_type=f32)
            y = jnp.concatenate([y[0:CC], y[CC:2 * CC]], axis=1)
            sd = cols[KS, ch, :]
            y = y + two(vb, ch) * jnp.concatenate([sd, sd], axis=1)
            x = two(qv, ch)
            hbuf[slot, ch, :] = x + (x - st["m"]) * st["r"] * y

        def norm():
            ybuf[slot, 0:D, :] = _ln(hbuf[slot]).astype(bf)

        parts = [stats]
        for d0 in range(0, D, CC):
            for d1 in range(d0, d0 + CC, FR):
                parts.append(functools.partial(mac, d1))
            parts.append(functools.partial(back, d0))
        parts.append(norm)
        return parts

    def out_copies(s):
        return tuple(
            pltpu.make_async_copy(ob.at[s, :, pl.ds(half * _B, _B)],
                                  out_hbm.at[:, pl.ds(pl.multiple_of(c * _B, _B), _B)],
                                  osem.at[2 * s + half])
            for half, c in enumerate((s, NB - 1 - s)))

    def mlp_parts(s, slot):
        st = {}

        def up(j):
            a = jnp.dot(w1t[j * FC:(j + 1) * FC, :], ybuf[slot], preferred_element_type=f32)
            gb[j * FC:(j + 1) * FC, :] = _gelu(a).astype(bf)

        def down(d0):
            ch = slice(d0, d0 + OC)
            o = jnp.dot(w2t[ch, :], gb[...], preferred_element_type=f32)
            b2 = cols[KS + 1, ch, :]
            ob[s, ch, :] = (o + (hbuf[slot, ch, :] + jnp.concatenate([b2, b2], axis=1))).astype(bf)

        parts = [functools.partial(up, j) for j in range(F // FC)]
        parts += [functools.partial(down, d0) for d0 in range(0, D, OC)]
        return parts
    def run(*lists):
        items = []
        for li, l in enumerate(lists):
            items += [((i + 0.5) / len(l), li, f) for i, f in enumerate(l)]
        for _, _, f in sorted(items, key=lambda t: t[:2]):
            f()

    q_cp.wait()
    run(conv_parts(0, 0))
    w2_cp.wait()
    w2t[...] = w2v[...]

    def p2(s, _):
        run(mlp_parts(s, s % 2), conv_parts(s + 1, (s + 1) % 2))
        for cp in out_copies(s):
            cp.start()
        return 0

    jax.lax.fori_loop(0, NS - 1, p2, 0)
    run(mlp_parts(NS - 1, (NS - 1) % 2))
    for cp in out_copies(NS - 1):
        cp.start()
    for s in range(NS):
        for cp in out_copies(s):
            cp.wait()


@jax.jit
def pallas_sequential_preLN__ssm_conv_h3__mixer_channel_mlp__prompt_kernel(
    A_q: jax.Array,
    A_k: jax.Array,
    A_v: jax.Array,
    A_shift_k: jax.Array,
    A_ssm_k: jax.Array,
    A_ssm_D: jax.Array,
    B_x: jax.Array,
    B_w1: jax.Array,
    B_b1: jax.Array,
    B_w2: jax.Array,
    B_b2: jax.Array,
):
    del B_x
    Bt, S, D = A_q.shape
    assert Bt == 1
    F = B_w1.shape[1]
    KS = A_shift_k.shape[1]
    DP = -(-(D + 16) // 128) * 128
    CH = 512
    NB = S // _B
    fwd, inv = _dft_mats()
    hbm = pl.BlockSpec(memory_space=pltpu.HBM)
    vm = pl.BlockSpec(memory_space=pltpu.VMEM)
    bf, f32 = jnp.bfloat16, jnp.float32
    out = pl.pallas_call(
        functools.partial(_kernel, S=S, D=D, DP=DP, F=F, KS=KS, CH=CH),
        in_specs=[hbm, hbm, hbm, vm, hbm, vm, hbm, vm, hbm, vm, vm, vm],
        out_specs=hbm,
        out_shape=jax.ShapeDtypeStruct((D, S), bf),
        scratch_shapes=[
            pltpu.VMEM((D, S), bf),
            pltpu.VMEM((D, S + _B), bf),
            pltpu.VMEM((D, S), bf),
            pltpu.VMEM((D, S), bf),
            pltpu.VMEM((DP, F), bf),
            pltpu.VMEM((F, DP), bf),
            pltpu.VMEM((D, F), bf),
            pltpu.VMEM((D, F), bf),
            pltpu.VMEM((F, 2 * _B), bf),
            pltpu.VMEM((128, DP), f32),
            pltpu.VMEM((KS + 2, D, _B), f32),
            pltpu.VMEM((NB, D, 2 * _B), f32),
            pltpu.VMEM((NB, D, 2 * _B), f32),
            pltpu.VMEM((2, D, 2 * _B), f32),
            pltpu.VMEM((2, D, 2 * _B), f32),
            pltpu.VMEM((2, DP, 2 * _B), bf),
            pltpu.VMEM((NB // 2, D, 2 * _B), bf),
            pltpu.SemaphoreType.DMA((3 * (S // CH) + 3,)),
            pltpu.SemaphoreType.DMA((NB,)),
        ],
        compiler_params=pltpu.CompilerParams(vmem_limit_bytes=100 * 1024 * 1024),
    )(A_q[0].T, A_k[0].T, A_v[0].T, A_shift_k.T, A_ssm_k,
      A_ssm_D, B_w1, B_b1, B_w2.T, B_b2,
      jnp.asarray(fwd, dtype=bf), jnp.asarray(inv, dtype=bf))
    return out.T[None]
```
